```python
import jax
import jax.numpy as jnp

def _softmax(x, axis=-1):
    return jax.nn.softmax(x, axis=axis)
def _gelu(x):
    return jax.nn.gelu(x, approximate=True)
def _silu(x):
    return jax.nn.silu(x)
def _sigmoid(x):
    return jax.nn.sigmoid(x)
def _layernorm(x, axis=-1, eps=1e-5):
    m = jnp.mean(x, axis=axis, keepdims=True)
    v = jnp.var(x, axis=axis, keepdims=True)
    return (x - m) / jnp.sqrt(v + eps)
def _scatter_add(tgt, idx, src, axis=0):
    return tgt.at[idx].add(src)
def _segment_sum(src, seg, n):
    return jax.ops.segment_sum(src, seg, n)
class _Rng:
    def __init__(self, key):
        self._k = key
    def _next(self):
        self._k, sub = jax.random.split(self._k)
        return sub
    def normal(self, shape):
        return jax.random.normal(self._next(), shape, dtype=jnp.bfloat16)
    def randint(self, lo, hi, shape):
        return jax.random.randint(self._next(), shape, lo, hi, dtype=jnp.int32)
    def uniform(self, shape, lo=0.0, hi=1.0):
        return jax.random.uniform(self._next(), shape, jnp.bfloat16, lo, hi)
    def permutation(self, n):
        return jax.random.permutation(self._next(), n)


kernel_name = 'sequential_preLN__sliding_block__glu_gated_glu__prompt'

def _fwd_setup_inputs():
    _rng = _Rng(jax.random.key(int.from_bytes(__import__("os").urandom(4), "little")))
    _w = (lambda a: (lambda t: t.astype(jnp.bfloat16) if jnp.issubdtype(t.dtype, jnp.floating) else t)(jnp.asarray(a)))
    def _A_setup():
        B, S, D = 1, 2048, 512
        return {
            "x": _w((lambda *s: _rng.normal(s) * 0.05)(B, S, D)),
            "wqkv": _w((lambda *s: _rng.normal(s) * 0.05)(D, 3 * D)),
            "wo": _w((lambda *s: _rng.normal(s) * 0.05)(D, D)),
        }
    _A_in = _A_setup()

    def _B_setup():
        B, S, D, F = 1, 2048, 512, 1376
        return {
            "x": _w((lambda *s: _rng.normal(s) * 0.05)(B, S, D)),
            "w_gate": _w((lambda *s: _rng.normal(s) * 0.05)(D, F)),
            "w_up": _w((lambda *s: _rng.normal(s) * 0.05)(D, F)),
            "w_down": _w((lambda *s: _rng.normal(s) * 0.05)(F, D)),
        }
    _B_in = _B_setup()

    return {
        "A_x": _A_in["x"],
        "A_wqkv": _A_in["wqkv"],
        "A_wo": _A_in["wo"],
        "B_x": _B_in["x"],
        "B_w_gate": _B_in["w_gate"],
        "B_w_up": _B_in["w_up"],
        "B_w_down": _B_in["w_down"],
    }

def _fwd_reference(A_x, A_wqkv, A_wo, B_x, B_w_gate, B_w_up, B_w_down):
    def _A_ref(x, wqkv, wo):
        B, S, D = x.shape
        H = 32; Dh = D // H; W = 256
        qkv = (lambda x, *d: x.transpose(*d))((x @ wqkv).reshape(B, S, 3, H, Dh), 2, 0, 3, 1, 4)
        q, k, v = qkv[0], qkv[1], qkv[2]
        scores = jnp.einsum("bhqd,bhkd->bhqk", q, k) * (Dh ** -0.5)
        idx = jnp.arange(S)
        mask = (idx[:, None] - idx[None, :] >= 0) & (idx[:, None] - idx[None, :] < W)
        scores = jnp.where(mask[None, None], scores, -1e9)
        p = _softmax(scores, axis=-1)
        o = jnp.einsum("bhqk,bhkd->bhqd", p, v)
        return (lambda x, *d: x.transpose(*d))(o, 0, 2, 1, 3).reshape(B, S, D) @ wo

    def _B_ref(x, w_gate, w_up, w_down):
        g = jnp.einsum("bsd,df->bsf", x, w_gate)
        u = jnp.einsum("bsd,df->bsf", x, w_up)
        h = _sigmoid(g) * u
        return jnp.einsum("bsf,fd->bsd", h, w_down)

    x = A_x
    h = x + _A_ref(_layernorm(x, axis=-1), A_wqkv, A_wo)
    h2 = h + _B_ref(_layernorm(h, axis=-1), B_w_gate, B_w_up, B_w_down)
    return h2


def setup_inputs():
    _inp = _fwd_setup_inputs()
    _gk = jax.random.fold_in(jax.random.key(int.from_bytes(__import__("os").urandom(4), "little")), 2**31 - 1)
    _shapes = [[1, 2048, 512]]
    _dtypes = ['bfloat16']
    _gks = jax.random.split(_gk, len(_shapes))
    _gs = [jax.random.normal(k, s, dtype=jnp.dtype(d)) * 0.05 for k, s, d in zip(_gks, _shapes, _dtypes)]
    _inp["grad_out"] = _gs[0]
    return _inp

def reference(A_x, A_wqkv, A_wo, B_w_gate, B_w_up, B_w_down, B_x, grad_out):
    _const = dict(B_x=B_x)
    def _f(*_d):
        return _fwd_reference(**{'A_x': _d[0], 'A_wqkv': _d[1], 'A_wo': _d[2], 'B_w_gate': _d[3], 'B_w_up': _d[4], 'B_w_down': _d[5], **_const})
    _out, _vjp = jax.vjp(_f, A_x, A_wqkv, A_wo, B_w_gate, B_w_up, B_w_down)
    _grads = _vjp(grad_out)
    _out0 = jnp.asarray(_out)
    return (_out0, *[jnp.asarray(_g) for _g in _grads])
```

```python
import functools

import jax
import jax.numpy as jnp
import jax.experimental.pallas as pl
import jax.experimental.pallas.tpu as pltpu

S, D, F = 2048, 512, 1376
H, DH, W = 32, 16, 256
QB = 128
KW = 3 * QB
PADK = 2 * QB
T = 512
NB = S // T
NSUB = T // QB
G = 4
HG = 8
EPS = 1e-5
SCALE = DH ** -0.5
BF = jnp.bfloat16
F32 = jnp.float32


def _dot(a, b):
    return jnp.dot(a, b, preferred_element_type=F32)


def _ln_fwd(x):
    m = jnp.mean(x, axis=-1, keepdims=True)
    c = x - m
    v = jnp.mean(c * c, axis=-1, keepdims=True)
    r = 1.0 / jnp.sqrt(v + EPS)
    return c * r, r


def _ln_bwd(dy, y, r):
    return r * (dy - jnp.mean(dy, axis=-1, keepdims=True)
                - y * jnp.mean(dy * y, axis=-1, keepdims=True))


def _kernel(x_ref, go_ref, wqkv_ref, wo_ref, wg_ref, wu_ref, wd_ref,
            y_ref, dx_ref, dwqkv_ref, dwo_ref, dwg_ref, dwu_ref, dwd_ref,
            wqkvT, woT, wgT, wuT, wdT,
            a_wqkv, a_wo, a_wg, a_wu, a_wdT,
            k_nat, v_nat, kT, vT, dk_acc, dv_acc,
            xn_s, r1_s, dh_s, dq_s,
            qT_c, q_c, oT_c, doT_c, e_c, linv_c):
    i = pl.program_id(0)

    @pl.when(i == 0)
    def _init():
        wqkvT[...] = wqkv_ref[...].astype(F32).T.astype(BF)
        woT[...] = wo_ref[...].astype(F32).T.astype(BF)
        wgT[...] = wg_ref[...].astype(F32).T.astype(BF)
        wuT[...] = wu_ref[...].astype(F32).T.astype(BF)
        wdT[...] = wd_ref[...].astype(F32).T.astype(BF)
        a_wqkv[...] = jnp.zeros_like(a_wqkv)
        a_wo[...] = jnp.zeros_like(a_wo)
        a_wg[...] = jnp.zeros_like(a_wg)
        a_wu[...] = jnp.zeros_like(a_wu)
        a_wdT[...] = jnp.zeros_like(a_wdT)
        k_nat[...] = jnp.zeros_like(k_nat)
        v_nat[...] = jnp.zeros_like(v_nat)
        kT[...] = jnp.zeros_like(kT)
        vT[...] = jnp.zeros_like(vT)
        dk_acc[...] = jnp.zeros_like(dk_acc)
        dv_acc[...] = jnp.zeros_like(dv_acc)

    row16 = jax.lax.broadcasted_iota(jnp.int32, (QB, QB), 0) // DH
    lane16 = jax.lax.broadcasted_iota(jnp.int32, (QB, QB), 1) // DH

    @pl.when(i < NB)
    def _main():
        r0 = pl.multiple_of(i * T, T)
        x = x_ref[...].astype(F32)
        xn, r1 = _ln_fwd(x)
        xn_s[pl.ds(r0, T), :] = xn
        r1_s[pl.ds(r0, T), :] = jnp.broadcast_to(r1, (T, 128))
        qkv = _dot(xn.astype(BF), wqkv_ref[...])
        q = qkv[:, 0:D] * SCALE
        k = qkv[:, D:2 * D]
        v = qkv[:, 2 * D:3 * D]
        q_c[...] = q.astype(BF)
        qT_c[...] = q.T.astype(BF)
        k_nat[pl.ds(PADK + r0, T), :] = k.astype(BF)
        v_nat[pl.ds(PADK + r0, T), :] = v.astype(BF)
        kT[:, pl.ds(PADK + r0, T)] = k.T.astype(BF)
        vT[:, pl.ds(PADK + r0, T)] = v.T.astype(BF)

        def att_fwd(sb, carry):
            c0 = pl.multiple_of(sb * QB, QB)
            k0 = pl.multiple_of(r0 + sb * QB, QB)
            rk = jax.lax.broadcasted_iota(jnp.int32, (KW, QB), 0)
            rq = jax.lax.broadcasted_iota(jnp.int32, (KW, QB), 1)
            valid = (rk > rq) & (rk <= rq + W) & (rk >= PADK - k0)
            for g in range(G):
                kg = k_nat[pl.ds(k0, KW), g * 128:(g + 1) * 128]
                qgT = qT_c[g * 128:(g + 1) * 128, pl.ds(c0, QB)]
                zero = jnp.zeros_like(qgT)
                wq = jnp.concatenate(
                    [jnp.where(row16 == h, qgT, zero) for h in range(HG)], axis=1)
                sT = _dot(kg, wq)
                for h in range(HG):
                    s = jnp.where(valid, sT[:, h * 128:(h + 1) * 128], -1e9)
                    m = jnp.max(s, axis=0, keepdims=True)
                    e = jnp.exp(s - m)
                    l = jnp.sum(e, axis=0, keepdims=True)
                    linv = 1.0 / l
                    eb = e.astype(BF)
                    e_c[sb, g, :, h * 128:(h + 1) * 128] = eb
                    hh = g * HG + h
                    linv_c[sb, hh:hh + 1, :] = linv
                    vth = vT[hh * DH:(hh + 1) * DH, pl.ds(k0, KW)]
                    oT_c[hh * DH:(hh + 1) * DH, pl.ds(c0, QB)] = _dot(vth, eb) * linv
            return carry

        jax.lax.fori_loop(0, NSUB, att_fwd, 0)

        oT = oT_c[...]
        o = oT.T.astype(BF)
        h = x + _dot(o, wo_ref[...])
        hn, r2 = _ln_fwd(h)
        hnb = hn.astype(BF)
        gg = _dot(hnb, wg_ref[...])
        uu = _dot(hnb, wu_ref[...])
        sg = jax.nn.sigmoid(gg)
        hhb = (sg * uu).astype(BF)
        y_ref[...] = (h + _dot(hhb, wd_ref[...])).astype(y_ref.dtype)

        dy = go_ref[...].astype(F32)
        dyb = go_ref[...]
        dhh = _dot(dyb, wdT[...])
        du = (dhh * sg).astype(BF)
        dg = (dhh * uu * sg * (1.0 - sg)).astype(BF)
        dyT = dy.T.astype(BF)
        hnT = hn.T.astype(BF)
        a_wdT[...] += _dot(dyT, hhb)
        a_wg[...] += _dot(hnT, dg)
        a_wu[...] += _dot(hnT, du)
        dhn = _dot(dg, wgT[...]) + _dot(du, wuT[...])
        dh = dy + _ln_bwd(dhn, hn, r2)
        dh_s[pl.ds(r0, T), :] = dh
        dhb = dh.astype(BF)
        a_wo[...] += _dot(oT.astype(BF), dhb)
        do = _dot(dhb, woT[...])
        doT_c[...] = do.T

        def att_bwd(sb, carry):
            c0 = pl.multiple_of(sb * QB, QB)
            k0 = pl.multiple_of(r0 + sb * QB, QB)
            for g in range(G):
                vg = v_nat[pl.ds(k0, KW), g * 128:(g + 1) * 128]
                doT_g = doT_c[g * 128:(g + 1) * 128, pl.ds(c0, QB)]
                oT_g = oT_c[g * 128:(g + 1) * 128, pl.ds(c0, QB)]
                prod = doT_g * oT_g
                linv_rows = jnp.concatenate(
                    [jnp.broadcast_to(linv_c[sb, g * HG + h:g * HG + h + 1, :], (DH, QB))
                     for h in range(HG)], axis=0)
                doTs = doT_g * linv_rows
                zero = jnp.zeros_like(doTs)
                wdo = jnp.concatenate(
                    [jnp.where(row16 == h, doTs, zero) for h in range(HG)], axis=1).astype(BF)
                dpT = _dot(vg, wdo)
                dos = doTs.T
                dostack = jnp.concatenate(
                    [jnp.where(lane16 == h, dos, zero) for h in range(HG)], axis=0).astype(BF)
                qg = q_c[pl.ds(c0, QB), g * 128:(g + 1) * 128]
                zb = jnp.zeros_like(qg)
                qstack = jnp.concatenate(
                    [jnp.where(lane16 == h, qg, zb) for h in range(HG)], axis=0)
                eb = e_c[sb, g]
                ds_parts = []
                for h in range(HG):
                    hh = g * HG + h
                    delta = jnp.sum(prod[h * DH:(h + 1) * DH, :], axis=0, keepdims=True)
                    delta = delta * linv_c[sb, hh:hh + 1, :]
                    ds = eb[:, h * 128:(h + 1) * 128].astype(F32) * (
                        dpT[:, h * 128:(h + 1) * 128] - delta)
                    dsb = ds.astype(BF)
                    ds_parts.append(dsb)
                    kth = kT[hh * DH:(hh + 1) * DH, pl.ds(k0, KW)]
                    dq_s[hh * DH:(hh + 1) * DH, pl.ds(r0 + c0, QB)] = _dot(kth, dsb) * SCALE
                dsT = jnp.concatenate(ds_parts, axis=1)
                dv_acc[pl.ds(k0, KW), g * 128:(g + 1) * 128] += _dot(eb, dostack)
                dk_acc[pl.ds(k0, KW), g * 128:(g + 1) * 128] += _dot(dsT, qstack)
            return carry

        jax.lax.fori_loop(0, NSUB, att_bwd, 0)

    @pl.when(i > 0)
    def _fin():
        p0 = pl.multiple_of((i - 1) * T, T)
        dq = dq_s[:, pl.ds(p0, T)].T
        dk = dk_acc[pl.ds(PADK + p0, T), :]
        dv = dv_acc[pl.ds(PADK + p0, T), :]
        dqkv = jnp.concatenate([dq, dk, dv], axis=1).astype(BF)
        xn = xn_s[pl.ds(p0, T), :]
        r1 = r1_s[pl.ds(p0, T), 0:1]
        a_wqkv[...] += _dot(xn.T.astype(BF), dqkv)
        dxn = _dot(dqkv, wqkvT[...])
        dx_ref[...] = (dh_s[pl.ds(p0, T), :] + _ln_bwd(dxn, xn, r1)).astype(dx_ref.dtype)

    @pl.when(i == NB)
    def _out():
        dwqkv_ref[...] = a_wqkv[...].astype(BF)
        dwo_ref[...] = a_wo[...].astype(BF)
        dwg_ref[...] = a_wg[...].astype(BF)
        dwu_ref[...] = a_wu[...].astype(BF)
        dwd_ref[...] = a_wdT[...].T.astype(BF)


@jax.jit
def pallas_sequential_preLN__sliding_block__glu_gated_glu__prompt_kernel(
    A_x, A_wqkv, A_wo, B_x, B_w_gate, B_w_up, B_w_down, grad_out,
):
    x = A_x.reshape(S, D)
    go = grad_out.reshape(S, D)

    cur = lambda i: (jnp.minimum(i, NB - 1), 0)
    prev = lambda i: (jnp.maximum(i - 1, 0), 0)
    whole = lambda shape: pl.BlockSpec(shape, lambda i: (0, 0))

    in_specs = [
        pl.BlockSpec((T, D), cur), pl.BlockSpec((T, D), cur),
        whole((D, 3 * D)), whole((D, D)), whole((D, F)), whole((D, F)), whole((F, D)),
    ]
    out_specs = [
        pl.BlockSpec((T, D), cur), pl.BlockSpec((T, D), prev),
        whole((D, 3 * D)), whole((D, D)), whole((D, F)), whole((D, F)), whole((F, D)),
    ]
    out_shape = [
        jax.ShapeDtypeStruct((S, D), BF), jax.ShapeDtypeStruct((S, D), BF),
        jax.ShapeDtypeStruct((D, 3 * D), BF), jax.ShapeDtypeStruct((D, D), BF),
        jax.ShapeDtypeStruct((D, F), BF), jax.ShapeDtypeStruct((D, F), BF),
        jax.ShapeDtypeStruct((F, D), BF),
    ]
    V = pltpu.VMEM
    scratch = [
        V((3 * D, D), BF), V((D, D), BF), V((F, D), BF), V((F, D), BF), V((D, F), BF),
        V((D, 3 * D), F32), V((D, D), F32), V((D, F), F32), V((D, F), F32), V((D, F), F32),
        V((S + PADK, D), BF), V((S + PADK, D), BF), V((D, S + PADK), BF), V((D, S + PADK), BF),
        V((S + PADK, D), F32), V((S + PADK, D), F32),
        V((S, D), F32), V((S, 128), F32), V((S, D), F32), V((D, S), F32),
        V((D, T), BF), V((T, D), BF), V((D, T), F32), V((D, T), F32),
        V((NSUB, G, KW, HG * QB), BF), V((NSUB, H, QB), F32),
    ]
    outs = pl.pallas_call(
        _kernel,
        grid=(NB + 1,),
        in_specs=in_specs,
        out_specs=out_specs,
        out_shape=out_shape,
        scratch_shapes=scratch,
        compiler_params=pltpu.CompilerParams(
            dimension_semantics=("arbitrary",),
            vmem_limit_bytes=120 * 1024 * 1024,
        ),
    )(x, go, A_wqkv, A_wo, B_w_gate, B_w_up, B_w_down)
    y, dx, dwqkv, dwo, dwg, dwu, dwd = outs
    return (y.reshape(1, S, D), dx.reshape(1, S, D), dwqkv, dwo, dwg, dwu, dwd)
```

```python
import jax
import jax.numpy as jnp
import jax.experimental.pallas as pl
import jax.experimental.pallas.tpu as pltpu

S, D, F = 2048, 512, 1376
H, DH, W = 32, 16, 256
QB = 128
KW = 3 * QB
PADK = 2 * QB
T = 256
NB = S // T
NSUB = T // QB
G = 4
HG = 8
NFT = -(-F // 128)
NPRE = 3
EPS = 1e-5
SCALE = DH ** -0.5
LOG2E = 1.4426950408889634
LN2 = 0.6931471805599453
NEG = -1e9
BF = jnp.bfloat16
F32 = jnp.float32


def _dot(a, b):
    return jnp.dot(a, b, preferred_element_type=F32)


def _dg(a, b, ca, cb):
    return jax.lax.dot_general(a, b, (((ca,), (cb,)), ((), ())), preferred_element_type=F32)


def _ln_fwd(x):
    m = jnp.mean(x, axis=-1, keepdims=True)
    c = x - m
    v = jnp.mean(c * c, axis=-1, keepdims=True)
    r = 1.0 / jnp.sqrt(v + EPS)
    return c * r, r


def _ln_bwd(dy, y, r):
    return r * (dy - jnp.mean(dy, axis=-1, keepdims=True)
                - y * jnp.mean(dy * y, axis=-1, keepdims=True))


def _kernel(x_ref, go_ref, wqkv_hbm, wo_hbm, wgT_hbm, wuT_hbm, wd_hbm,
            y_ref, dx_ref, dwqkv_hbm, dwo_hbm, dwgT_hbm, dwuT_hbm, dwd_hbm,
            wqkv_ref, wo_ref, wgT_ref, wuT_ref, wd_ref,
            o_wqkv, o_wo, o_wg, o_wu, o_wd, sem_in, sem_out,
            a_wqkvT, a_wo, a_wg, a_wu, a_wd,
            k_nat, v_nat, kT, vT, dkT, dvT,
            xn_s, r1_s, dh_s, dqT,
            qT_c, oT_c, doT_c, e_c, c_c, dhh_c):
    i = pl.program_id(0)

    w_pairs = ((wqkv_hbm, wqkv_ref), (wo_hbm, wo_ref), (wgT_hbm, wgT_ref),
               (wuT_hbm, wuT_ref), (wd_hbm, wd_ref))
    o_pairs = ((o_wqkv, dwqkv_hbm), (o_wo, dwo_hbm), (o_wg, dwgT_hbm),
               (o_wu, dwuT_hbm), (o_wd, dwd_hbm))

    def in_copy(j):
        return pltpu.make_async_copy(w_pairs[j][0], w_pairs[j][1], sem_in.at[j])

    def out_copy(j):
        return pltpu.make_async_copy(o_pairs[j][0], o_pairs[j][1], sem_out.at[j])

    def wait_in(*js):
        @pl.when(i == 0)
        def _():
            for j in js:
                in_copy(j).wait()

    @pl.when(i == 0)
    def _init():
        for j in (4, 0, 1, 2, 3):
            in_copy(j).start()
        a_wqkvT[...] = jnp.zeros_like(a_wqkvT)
        a_wo[...] = jnp.zeros_like(a_wo)
        a_wg[...] = jnp.zeros_like(a_wg)
        a_wu[...] = jnp.zeros_like(a_wu)
        a_wd[...] = jnp.zeros_like(a_wd)
        k_nat[0:PADK, :] = jnp.zeros((PADK, D), BF)
        v_nat[0:PADK, :] = jnp.zeros((PADK, D), BF)
        kT[:, 0:PADK] = jnp.zeros((D, PADK), BF)
        vT[:, 0:PADK] = jnp.zeros((D, PADK), BF)
        dkT[...] = jnp.zeros_like(dkT)
        dvT[...] = jnp.zeros_like(dvT)

    row16 = jax.lax.broadcasted_iota(jnp.int32, (QB, QB), 0) // DH

    @pl.when(i < NB)
    def _main():
        r0 = pl.multiple_of(i * T, T)
        def dhh_tile(n):
            f0, f1 = n * 128, min((n + 1) * 128, F)
            dhh_c[:, f0:f1] = _dg(go_ref[...], wd_ref[f0:f1, :], 1, 1)

        wait_in(4)
        for n in range(NPRE):
            dhh_tile(n)
        x = x_ref[...].astype(F32)
        xn, r1 = _ln_fwd(x)
        xn_s[pl.ds(r0, T), :] = xn
        r1_s[pl.ds(r0, T), :] = jnp.broadcast_to(r1, (T, 128))
        wait_in(0)
        qkv = _dot(xn.astype(BF), wqkv_ref[...])
        q = qkv[:, 0:D] * (SCALE * LOG2E)
        k = qkv[:, D:2 * D]
        v = qkv[:, 2 * D:3 * D]
        qT_c[...] = q.T.astype(BF)
        k_nat[pl.ds(PADK + r0, T), :] = k.astype(BF)
        v_nat[pl.ds(PADK + r0, T), :] = v.astype(BF)
        kT[:, pl.ds(PADK + r0, T)] = k.T.astype(BF)
        vT[:, pl.ds(PADK + r0, T)] = v.T.astype(BF)

        def att_fwd(sb, carry):
            c0 = pl.multiple_of(sb * QB, QB)
            k0 = pl.multiple_of(r0 + sb * QB, QB)
            rk = jax.lax.broadcasted_iota(jnp.int32, (QB, QB), 0)
            rq = jax.lax.broadcasted_iota(jnp.int32, (QB, QB), 1)
            upper = rk > rq
            v0 = k0 >= 2 * QB
            v1 = k0 >= QB
            def scores(qd):
                g, half = divmod(qd, 2)
                kg = k_nat[pl.ds(k0, KW), g * 128:(g + 1) * 128]
                qgT = qT_c[g * 128:(g + 1) * 128, pl.ds(c0, QB)]
                zero = jnp.zeros_like(qgT)
                wq = jnp.concatenate(
                    [jnp.where(row16 == h, qgT, zero) for h in range(4 * half, 4 * half + 4)],
                    axis=1)
                return _dot(kg, wq)

            sT_next = scores(0)
            for qd in range(2 * G):
                g, half = divmod(qd, 2)
                sT = sT_next
                if qd + 1 < 2 * G:
                    sT_next = scores(qd + 1)
                n = NPRE + sb * 2 * G + qd
                if n < NFT:
                    dhh_tile(n)
                for h4 in range(4):
                    h = 4 * half + h4
                    hh = g * HG + h
                    cols = slice(h * 128, (h + 1) * 128)
                    c4 = slice(h4 * 128, (h4 + 1) * 128)
                    st = [jnp.where(upper, sT[0:QB, c4], NEG),
                          sT[QB:2 * QB, c4],
                          jnp.where(upper, NEG, sT[2 * QB:3 * QB, c4])]
                    mt, lt, ot = [], [], []
                    for t in range(3):
                        m_t = jnp.max(st[t], axis=0, keepdims=True)
                        e = jnp.exp2(st[t] - m_t)
                        lt.append(jnp.sum(e, axis=0, keepdims=True))
                        mt.append(m_t)
                        e_c[sb, g, t * QB:(t + 1) * QB, cols] = e
                        eb = e.astype(BF)
                        vth = vT[hh * DH:(hh + 1) * DH, pl.ds(k0 + t * QB, QB)]
                        ot.append(_dot(vth, eb))
                    m0 = jnp.where(v0, mt[0], NEG)
                    m1 = jnp.where(v1, mt[1], NEG)
                    m = jnp.maximum(jnp.maximum(m0, m1), mt[2])
                    sc = [jnp.where(v0, jnp.exp2(m0 - m), 0.0),
                          jnp.where(v1, jnp.exp2(m1 - m), 0.0),
                          jnp.exp2(mt[2] - m)]
                    linv = 1.0 / (sc[0] * lt[0] + sc[1] * lt[1] + sc[2] * lt[2])
                    acc = None
                    for t in range(3):
                        c_t = sc[t] * linv
                        c_c[sb, t, hh:hh + 1, :] = c_t
                        acc = ot[t] * c_t if acc is None else acc + ot[t] * c_t
                    oT_c[hh * DH:(hh + 1) * DH, pl.ds(c0, QB)] = acc
            return carry

        for sb in range(NSUB):
            att_fwd(sb, 0)

        wait_in(1, 2, 3)
        oTb = oT_c[...].astype(BF)
        h = x + _dg(oTb, wo_ref[...], 0, 0)
        hn, r2 = _ln_fwd(h)
        hnb = hn.astype(BF)
        dyb = go_ref[...]
        gg = _dg(hnb, wgT_ref[...], 1, 1)
        uu = _dg(hnb, wuT_ref[...], 1, 1)
        dhh = dhh_c[...]
        sg = jax.nn.sigmoid(gg)
        hhb = (sg * uu).astype(BF)
        y_ref[...] = (h + _dot(hhb, wd_ref[...])).astype(y_ref.dtype)
        du = (dhh * sg).astype(BF)
        dg = (dhh * uu * sg * (1.0 - sg)).astype(BF)
        dhn = _dot(dg, wgT_ref[...]) + _dot(du, wuT_ref[...])
        a_wd[...] += _dg(hhb, dyb, 0, 0)
        a_wg[...] += _dg(dg, hnb, 0, 0)
        a_wu[...] += _dg(du, hnb, 0, 0)
        dh = dyb.astype(F32) + _ln_bwd(dhn, hn, r2)
        dh_s[pl.ds(r0, T), :] = dh
        dhb = dh.astype(BF)
        doT_c[...] = _dg(wo_ref[...], dhb, 1, 1)
        a_wo[...] += _dot(oTb, dhb)

        @pl.when(i == NB - 1)
        def _flush():
            o_wo[...] = a_wo[...].astype(BF)
            o_wg[...] = a_wg[...].astype(BF)
            o_wu[...] = a_wu[...].astype(BF)
            o_wd[...] = a_wd[...].astype(BF)
            for j in range(1, 5):
                out_copy(j).start()

        def att_bwd(sb, carry):
            c0 = pl.multiple_of(sb * QB, QB)
            k0 = pl.multiple_of(r0 + sb * QB, QB)
            def dscores(qd):
                g, half = divmod(qd, 2)
                vg = v_nat[pl.ds(k0, KW), g * 128:(g + 1) * 128]
                doTb = doT_c[g * 128:(g + 1) * 128, pl.ds(c0, QB)].astype(BF)
                zero = jnp.zeros_like(doTb)
                wdo = jnp.concatenate(
                    [jnp.where(row16 == h, doTb, zero) for h in range(4 * half, 4 * half + 4)],
                    axis=1)
                return _dot(vg, wdo)

            dp_next = dscores(0)
            for qd in range(2 * G):
                g, half = divmod(qd, 2)
                dpT = dp_next
                if qd + 1 < 2 * G:
                    dp_next = dscores(qd + 1)
                for h4 in range(4):
                    h = 4 * half + h4
                    hh = g * HG + h
                    cols = slice(h * 128, (h + 1) * 128)
                    c4 = slice(h4 * 128, (h4 + 1) * 128)
                    rows = slice(hh * DH, (hh + 1) * DH)
                    doT_h = doT_c[rows, pl.ds(c0, QB)]
                    oT_h = oT_c[rows, pl.ds(c0, QB)]
                    qT_h = qT_c[rows, pl.ds(c0, QB)].astype(F32) * LN2
                    delta = jnp.sum(doT_h * oT_h, axis=0, keepdims=True)
                    dq = None
                    for t in range(3):
                        c_t = c_c[sb, t, hh:hh + 1, :]
                        e = e_c[sb, g, t * QB:(t + 1) * QB, cols]
                        eb = e.astype(BF)
                        ds = e * (dpT[t * QB:(t + 1) * QB, c4] - delta)
                        dsb = ds.astype(BF)
                        kth = kT[rows, pl.ds(k0 + t * QB, QB)]
                        part = _dot(kth, dsb) * c_t
                        dq = part if dq is None else dq + part
                        dvT[rows, pl.ds(k0 + t * QB, QB)] += _dot(
                            (doT_h * c_t).astype(BF), e.T.astype(BF))
                        dkT[rows, pl.ds(k0 + t * QB, QB)] += _dg(
                            (qT_h * c_t).astype(BF), dsb, 1, 1)
                    dqT[rows, pl.ds(r0 + c0, QB)] = dq * SCALE
            return carry

        for sb in range(NSUB):
            att_bwd(sb, 0)

    @pl.when(i > 0)
    def _fin():
        p0 = pl.multiple_of((i - 1) * T, T)
        dqkvT = jnp.concatenate(
            [dqT[:, pl.ds(p0, T)], dkT[:, pl.ds(PADK + p0, T)], dvT[:, pl.ds(PADK + p0, T)]],
            axis=0).astype(BF)
        xn = xn_s[pl.ds(p0, T), :]
        r1 = r1_s[pl.ds(p0, T), 0:1]
        a_wqkvT[...] += _dot(dqkvT, xn.astype(BF))

        @pl.when(i == NB)
        def _out():
            o_wqkv[...] = a_wqkvT[...].T.astype(BF)
            out_copy(0).start()

        dxn = _dg(dqkvT, wqkv_ref[...], 0, 1)
        dx_ref[...] = (dh_s[pl.ds(p0, T), :] + _ln_bwd(dxn, xn, r1)).astype(dx_ref.dtype)

    @pl.when(i == NB)
    def _drain():
        for j in range(5):
            out_copy(j).wait()


@jax.jit
def pallas_sequential_preLN__sliding_block__glu_gated_glu__prompt_kernel(
    A_x, A_wqkv, A_wo, B_x, B_w_gate, B_w_up, B_w_down, grad_out,
):
    x = A_x.reshape(S, D)
    go = grad_out.reshape(S, D)

    cur = lambda i: (jnp.minimum(i, NB - 1), 0)
    prev = lambda i: (jnp.maximum(i - 1, 0), 0)
    hbm = pl.BlockSpec(memory_space=pl.ANY)

    in_specs = [
        pl.BlockSpec((T, D), cur), pl.BlockSpec((T, D), cur),
        hbm, hbm, hbm, hbm, hbm,
    ]
    out_specs = [
        pl.BlockSpec((T, D), cur), pl.BlockSpec((T, D), prev),
        hbm, hbm, hbm, hbm, hbm,
    ]
    out_shape = [
        jax.ShapeDtypeStruct((S, D), BF), jax.ShapeDtypeStruct((S, D), BF),
        jax.ShapeDtypeStruct((D, 3 * D), BF), jax.ShapeDtypeStruct((D, D), BF),
        jax.ShapeDtypeStruct((F, D), BF), jax.ShapeDtypeStruct((F, D), BF),
        jax.ShapeDtypeStruct((F, D), BF),
    ]
    V = pltpu.VMEM
    scratch = [
        V((D, 3 * D), BF), V((D, D), BF), V((F, D), BF), V((F, D), BF), V((F, D), BF),
        V((D, 3 * D), BF), V((D, D), BF), V((F, D), BF), V((F, D), BF), V((F, D), BF),
        pltpu.SemaphoreType.DMA((5,)), pltpu.SemaphoreType.DMA((5,)),
        V((3 * D, D), F32), V((D, D), F32), V((F, D), F32), V((F, D), F32), V((F, D), F32),
        V((S + PADK, D), BF), V((S + PADK, D), BF), V((D, S + PADK), BF), V((D, S + PADK), BF),
        V((D, S + PADK), F32), V((D, S + PADK), F32),
        V((S, D), F32), V((S, 128), F32), V((S, D), F32), V((D, S), F32),
        V((D, T), BF), V((D, T), F32), V((D, T), F32),
        V((NSUB, G, KW, HG * QB), F32), V((NSUB, 3, H, QB), F32), V((T, F), F32),
    ]
    outs = pl.pallas_call(
        _kernel,
        grid=(NB + 1,),
        in_specs=in_specs,
        out_specs=out_specs,
        out_shape=out_shape,
        scratch_shapes=scratch,
        compiler_params=pltpu.CompilerParams(
            dimension_semantics=("arbitrary",),
            vmem_limit_bytes=120 * 1024 * 1024,
        ),
    )(x, go, A_wqkv, A_wo, B_w_gate.T, B_w_up.T, B_w_down)
    y, dx, dwqkv, dwo, dwgT, dwuT, dwd = outs
    return (y.reshape(1, S, D), dx.reshape(1, S, D), dwqkv, dwo, dwgT.T, dwuT.T, dwd)
```
